```python
import jax
import jax.numpy as jnp

def _softmax(x, axis=-1):
    return jax.nn.softmax(x, axis=axis)
def _gelu(x):
    return jax.nn.gelu(x, approximate=True)
def _silu(x):
    return jax.nn.silu(x)
def _sigmoid(x):
    return jax.nn.sigmoid(x)
def _layernorm(x, axis=-1, eps=1e-5):
    m = jnp.mean(x, axis=axis, keepdims=True)
    v = jnp.var(x, axis=axis, keepdims=True)
    return (x - m) / jnp.sqrt(v + eps)
def _scatter_add(tgt, idx, src, axis=0):
    return tgt.at[idx].add(src)
def _segment_sum(src, seg, n):
    return jax.ops.segment_sum(src, seg, n)
class _Rng:
    def __init__(self, key):
        self._k = key
    def _next(self):
        self._k, sub = jax.random.split(self._k)
        return sub
    def normal(self, shape):
        return jax.random.normal(self._next(), shape, dtype=jnp.bfloat16)
    def randint(self, lo, hi, shape):
        return jax.random.randint(self._next(), shape, lo, hi, dtype=jnp.int32)
    def uniform(self, shape, lo=0.0, hi=1.0):
        return jax.random.uniform(self._next(), shape, jnp.bfloat16, lo, hi)
    def permutation(self, n):
        return jax.random.permutation(self._next(), n)


kernel_name = 'concat_heads__gqa_block_cached__mha_block_cached__near_ridge'

def setup_inputs():
    _rng = _Rng(jax.random.key(int.from_bytes(__import__("os").urandom(4), "little")))
    _w = (lambda a: (lambda t: t.astype(jnp.bfloat16) if jnp.issubdtype(t.dtype, jnp.floating) else t)(jnp.asarray(a)))
    def _A_setup():
        B, Sq, D = 16, 160, 640
        Hq, Hkv, Sk, Dh = 32, 32, 512, 192
        assert Hq % Hkv == 0, (Hq, Hkv)
        return {
            "x": _w((lambda *s: _rng.normal(s) * 0.05)(B, Sq, D)),
            "k_cache": _w((lambda *s: _rng.normal(s) * 0.05)(B, Hkv, Sk, Dh)),
            "v_cache": _w((lambda *s: _rng.normal(s) * 0.05)(B, Hkv, Sk, Dh)),
            "wq": _w((lambda *s: _rng.normal(s) * 0.05)(D, Hq * Dh) * (D ** -0.5)),
            "wo": _w((lambda *s: _rng.normal(s) * 0.05)(Hq * Dh, D) * ((Hq * Dh) ** -0.5)),
        }
    _A_in = _A_setup()

    def _B_setup():
        B, Sq, D = 16, 160, 640
        H, Sk, Dh = 32, 512, 192
        return {
            "x": _w((lambda *s: _rng.normal(s) * 0.05)(B, Sq, D)),
            "k_cache": _w((lambda *s: _rng.normal(s) * 0.05)(B, H, Sk, Dh)),
            "v_cache": _w((lambda *s: _rng.normal(s) * 0.05)(B, H, Sk, Dh)),
            "wq": _w((lambda *s: _rng.normal(s) * 0.05)(D, H * Dh) * (D ** -0.5)),
            "wo": _w((lambda *s: _rng.normal(s) * 0.05)(H * Dh, D) * ((H * Dh) ** -0.5)),
        }
    _B_in = _B_setup()

    return {
        "A_x": _A_in["x"],
        "A_k_cache": _A_in["k_cache"],
        "A_v_cache": _A_in["v_cache"],
        "A_wq": _A_in["wq"],
        "A_wo": _A_in["wo"],
        "B_x": _B_in["x"],
        "B_k_cache": _B_in["k_cache"],
        "B_v_cache": _B_in["v_cache"],
        "B_wq": _B_in["wq"],
        "B_wo": _B_in["wo"],
    }

def reference(A_x, A_k_cache, A_v_cache, A_wq, A_wo, B_x, B_k_cache, B_v_cache, B_wq, B_wo):
    def _A_ref(x, k_cache, v_cache, wq, wo):
        B, Sq, D = x.shape
        Hq, Dh = 32, 192
        Hkv = k_cache.shape[1]
        rep = Hq // Hkv
        q = (lambda x, *d: x.transpose(*d))((x @ wq).reshape(B, Sq, Hq, Dh), 0, 2, 1, 3)
        k = jnp.repeat(k_cache, rep, axis=1)
        v = jnp.repeat(v_cache, rep, axis=1)
        scores = jnp.einsum("bhqd,bhkd->bhqk", q, k) * (Dh ** -0.5)
        p = _softmax(scores, axis=-1)
        o = jnp.einsum("bhqk,bhkd->bhqd", p, v)
        return (lambda x, *d: x.transpose(*d))(o, 0, 2, 1, 3).reshape(B, Sq, Hq * Dh) @ wo

    def _B_ref(x, k_cache, v_cache, wq, wo):
        B, Sq, D = x.shape
        H, Dh = 32, 192
        q = (lambda x, *d: x.transpose(*d))((x @ wq).reshape(B, Sq, H, Dh), 0, 2, 1, 3)
        scores = jnp.einsum("bhqd,bhkd->bhqk", q, k_cache) * (Dh ** -0.5)
        p = _softmax(scores, axis=-1)
        o = jnp.einsum("bhqk,bhkd->bhqd", p, v_cache)
        return (lambda x, *d: x.transpose(*d))(o, 0, 2, 1, 3).reshape(B, Sq, H * Dh) @ wo

    a = _A_ref(A_x, A_k_cache, A_v_cache, A_wq, A_wo)
    b = _B_ref(B_x, B_k_cache, B_v_cache, B_wq, B_wo)
    return jnp.concatenate([a, b], axis=-1)
```

```python
import jax
import jax.numpy as jnp
import numpy as np
from jax import lax
from jax.experimental import pallas as pl
from jax.experimental.pallas import tpu as pltpu

_NT = (((1,), (1,)), ((), ()))
_HG = 8


@jax.jit
def pallas_concat_heads__gqa_block_cached__mha_block_cached__near_ridge_kernel(
    A_x, A_k_cache, A_v_cache, A_wq, A_wo,
    B_x, B_k_cache, B_v_cache, B_wq, B_wo,
):
    B, SQ, D = A_x.shape
    _, H, SK, DH = A_k_cache.shape
    NP = _HG // 2
    NG = H // _HG
    C = float(DH ** -0.5 * np.log2(np.e))

    def kern(xa, ka, va, wqa, woa, xb, kb, vb, wqb, wob, o_ref, acc):
        g = pl.program_id(0)
        b = pl.program_id(1)
        lane = lax.broadcasted_iota(jnp.int32, (SQ, 128), 1)
        lo = lane < 64

        def qproj(x, wq):
            return jnp.dot(x[0], wq[...], preferred_element_type=jnp.float32) * C

        def scores(q, k, p):
            t0 = q[:, p * 384:p * 384 + 128].astype(jnp.bfloat16)
            t1 = q[:, p * 384 + 128:p * 384 + 256]
            t2 = q[:, p * 384 + 256:p * 384 + 384].astype(jnp.bfloat16)
            t1a = jnp.where(lo, t1, 0.0).astype(jnp.bfloat16)
            t1b = jnp.where(lo, 0.0, t1).astype(jnp.bfloat16)
            s0 = jnp.dot(jnp.concatenate([t0, t1a], axis=1), k[0, p, 0:256, :],
                         preferred_element_type=jnp.float32)
            s1 = jnp.dot(jnp.concatenate([t1b, t2], axis=1), k[0, p, 128:384, :],
                         preferred_element_type=jnp.float32)
            return s0, s1

        def softmax(s):
            m = jnp.max(s, axis=1, keepdims=True)
            e = jnp.exp2(s - m)
            l = jnp.sum(e, axis=1, keepdims=True)
            return e.astype(jnp.bfloat16), 1.0 / l

        def pv(p0, r0, p1, r1, v, p):
            o0 = lax.dot_general(p0, v[0, p, 0:256, :], _NT,
                                 preferred_element_type=jnp.float32) * r0
            o1 = lax.dot_general(p1, v[0, p, 128:384, :], _NT,
                                 preferred_element_type=jnp.float32) * r1
            mid = jnp.where(lo, o0[:, 128:256], o1[:, 0:128])
            return jnp.concatenate([o0[:, 0:128], mid, o1[:, 128:256]],
                                   axis=1).astype(jnp.bfloat16)

        qa = qproj(xa, wqa)
        qb = qproj(xb, wqb)
        units = [(qa, ka, va, p) for p in range(NP)] + [(qb, kb, vb, p) for p in range(NP)]
        ps = []
        for (q, k, v, p) in units:
            s0, s1 = scores(q, k, p)
            ps.append(softmax(s0) + softmax(s1))
        os_ = [pv(*pp, v, p) for (q, k, v, p), pp in zip(units, ps)]
        oa = jnp.concatenate(os_[:NP], axis=1)
        ob = jnp.concatenate(os_[NP:], axis=1)
        ra = jnp.dot(oa, woa[...], preferred_element_type=jnp.float32)
        rb = jnp.dot(ob, wob[...], preferred_element_type=jnp.float32)
        first = g == 0
        ta = jnp.where(first, 0.0, acc[b, :, 0:D]) + ra
        tb = jnp.where(first, 0.0, acc[b, :, D:2 * D]) + rb
        acc[b, :, 0:D] = ta
        acc[b, :, D:2 * D] = tb
        o_ref[0, :, 0:D] = ta.astype(jnp.bfloat16)
        o_ref[0, :, D:2 * D] = tb.astype(jnp.bfloat16)

    def t(a):
        return jnp.swapaxes(a, 2, 3).reshape(B, H // 2, 2 * DH, SK)

    xs = pl.BlockSpec((1, SQ, D), lambda g, b: (b, 0, 0))
    ks = pl.BlockSpec((1, NP, 2 * DH, SK), lambda g, b: (b, g, 0, 0))
    wqs = pl.BlockSpec((D, _HG * DH), lambda g, b: (0, g))
    wos = pl.BlockSpec((_HG * DH, D), lambda g, b: (g, 0))
    return pl.pallas_call(
        kern,
        grid=(NG, B),
        in_specs=[xs, ks, ks, wqs, wos] * 2,
        out_specs=pl.BlockSpec((1, SQ, 2 * D),
                               lambda g, b: (jnp.where(g == NG - 1, b, 0), 0, 0)),
        out_shape=jax.ShapeDtypeStruct((B, SQ, 2 * D), jnp.bfloat16),
        scratch_shapes=[pltpu.VMEM((B, SQ, 2 * D), jnp.float32)],
        compiler_params=pltpu.CompilerParams(
            dimension_semantics=("arbitrary", "arbitrary"),
            vmem_limit_bytes=100 * 2 ** 20),
    )(A_x, t(A_k_cache), t(A_v_cache), A_wq, A_wo,
      B_x, t(B_k_cache), t(B_v_cache), B_wq, B_wo)
```

```python
import functools
import jax
import jax.numpy as jnp
import numpy as np
from jax import lax
from jax.experimental import pallas as pl
from jax.experimental.pallas import tpu as pltpu

NT = (((1,), (1,)), ((), ()))


def make(HG=2, BB=4, NS=4, RG=1, RB=1, order="qqsspp", rorder="qqsspp", osplit=1, flags=None, frac=1):
    B, SQ, D, H, SK, DH = 16, 160, 640, 32, 512, 192
    NP = HG // 2
    NG_ALL = H // HG
    NG = NG_ALL // frac
    NB = B // BB
    NIT = NG * NB
    LB = NB.bit_length() - 1
    assert 1 << LB == NB and NS in (2, 4) and BB % RB == 0
    RPB = BB // RB
    LR = RPB.bit_length() - 1
    W = HG * DH
    C = float(DH ** -0.5 * np.log2(np.e))
    f32, bf16 = jnp.float32, jnp.bfloat16

    def dot(a, b):
        return jnp.dot(a, b, preferred_element_type=f32)

    def nt(a, b):
        return lax.dot_general(a, b, NT, preferred_element_type=f32)

    def kern(xa, ka, va, wqa, woa, xb, kb, vb, wqb, wob, o_hbm,
             xs_a, ks_a, vs_a, wqs_a, wos_a, xs_b, ks_b, vs_b, wqs_b, wos_b,
             acc, obuf, sem, rsem, xsem, wsem, osem):
        hbm = ((xa, ka, va, wqa, woa), (xb, kb, vb, wqb, wob))
        vm = ((xs_a, ks_a, vs_a, wqs_a, wos_a), (xs_b, ks_b, vs_b, wqs_b, wos_b))

        def x_cps(r):
            rows = pl.ds(r * (RB * SQ), RB * SQ) if isinstance(r, int) else pl.ds(pl.multiple_of(r * (RB * SQ), RB * SQ), RB * SQ)
            return [pltpu.make_async_copy(hbm[br][0].at[rows], vm[br][0].at[rows], xsem.at[br, r]) for br in range(2)]

        def kv_cps(it):
            g = it >> LB
            bi = it & (NB - 1)
            s = it & (NS - 1)
            return [pltpu.make_async_copy(hbm[br][kv].at[pl.ds(bi * BB, BB), g], vm[br][kv].at[s], sem.at[br, kv - 1, s])
                    for kv in (1, 2) for br in range(2)]

        def rkv_cps(r):
            it = r >> LR
            j = r & (RPB - 1)
            g = it >> LB
            bi = it & (NB - 1)
            s = it & (NS - 1)
            return [pltpu.make_async_copy(hbm[br][kv].at[pl.ds(bi * BB + j * RB, RB), g],
                                          vm[br][kv].at[s, pl.ds(j * RB, RB)], rsem.at[br, kv - 1, s, j])
                    for kv in (1, 2) for br in range(2)]

        def w_cps(g):
            s = g & 1
            col = pl.ds(g * W, W) if isinstance(g, int) else pl.ds(pl.multiple_of(g * W, W), W)
            return ([pltpu.make_async_copy(hbm[br][3].at[:, col], vm[br][3].at[s], wsem.at[br, 0, s]) for br in range(2)]
                    + [pltpu.make_async_copy(hbm[br][4].at[g], vm[br][4].at[s], wsem.at[br, 1, s]) for br in range(2)])

        OB = BB // osplit

        def o_cp(bi, br, j):
            rows = OB * SQ
            return pltpu.make_async_copy(
                obuf.at[bi & 1, br, pl.ds(j * rows, rows)],
                o_hbm.at[pl.ds(pl.multiple_of(bi * (BB * SQ) + j * rows, rows), rows), pl.ds(br * D, D)],
                osem.at[bi & 1, br, j])

        def compute(nb, s, j0, b0, ws, order, mid, osplit, emit):
            lane = lax.broadcasted_iota(jnp.int32, (SQ, 128), 1)
            lo = lane < 64
            m = nb * SQ

            def scores(q, br, b, p):
                k = vm[br][1]
                q = q[b * SQ:(b + 1) * SQ, p * 384:(p + 1) * 384]
                t0 = q[:, 0:128].astype(bf16)
                t1 = q[:, 128:256]
                t2 = q[:, 256:384].astype(bf16)
                t1a = jnp.where(lo, t1, 0.0).astype(bf16)
                t1b = jnp.where(lo, 0.0, t1).astype(bf16)
                s0 = dot(jnp.concatenate([t0, t1a], axis=1), k[s, j0 + b, p, 0:256, :])
                s1 = dot(jnp.concatenate([t1b, t2], axis=1), k[s, j0 + b, p, 128:384, :])
                return s0, s1

            def softmax(sc):
                mx = jnp.max(sc, axis=1, keepdims=True)
                e = jnp.exp2(sc - mx)
                l = jnp.sum(e, axis=1, keepdims=True)
                return e.astype(bf16), 1.0 / l

            def pv(p0, r0, p1, r1, br, b, p):
                v = vm[br][2]
                a0 = nt(p0, v[s, j0 + b, p, 0:128, :]) * r0
                m0 = nt(v[s, j0 + b, p, 128:192, :], p0[0:128])
                a2 = nt(p1, v[s, j0 + b, p, 256:384, :]) * r1
                m1 = nt(v[s, j0 + b, p, 192:256, :], p1[0:128])
                cn = nt(jnp.concatenate([p0[128:160], p1[128:160]], axis=0), v[s, j0 + b, p, 128:256, :])
                mt = jnp.concatenate([m0, m1], axis=0).T
                cm = jnp.where(lo[0:32], cn[0:32], cn[32:64])
                mid_ = jnp.concatenate([mt, cm], axis=0) * jnp.where(lo, r0, r1)
                return jnp.concatenate([a0, mid_, a2], axis=1).astype(bf16)

            qs, ps, os_ = {}, {}, {}

            def do_q(br):
                qs[br] = dot(vm[br][0][pl.ds(pl.multiple_of(b0 * SQ, SQ), m)], vm[br][3][ws]) * C

            def do_s(br):
                for b in range(nb):
                    for p in range(NP):
                        s0, s1 = scores(qs[br], br, b, p)
                        ps[br, b, p] = softmax(s0) + softmax(s1)

            def do_p(br):
                os_[br] = jnp.concatenate([
                    jnp.concatenate([pv(*ps[br, b, p], br, b, p) for p in range(NP)], axis=1)
                    for b in range(nb)], axis=0)

            def do_o(br):
                mo = m // osplit
                for j in range(osplit):
                    rows = pl.ds(pl.multiple_of(b0 * SQ + j * mo, SQ), mo)
                    t = acc[br, rows] + dot(os_[br][j * mo:(j + 1) * mo], vm[br][4][ws])
                    acc[br, rows] = t
                    emit(br, j, t)

            fn = dict(q=do_q, s=do_s, p=do_p, o=do_o)
            seqs = dict(qqsspp="q0 m q1 s0 s1 p0 p1 o0 o1", qsqp="q0 m s0 q1 p0 s1 o0 p1 o1",
                        seq="q0 m s0 p0 o0 q1 s1 p1 o1", qqspso="q0 m q1 s0 p0 s1 o0 p1 o1",
                        qsqsp="q0 m s0 q1 s1 p0 o0 p1 o1")
            for tok in seqs[order].split():
                if tok == "m":
                    mid()
                else:
                    fn[tok[0]](int(tok[1]))

        NR = RG * NB * RPB
        LOOK = (NS - 1) * RPB
        for c in w_cps(0) + x_cps(0) + (rkv_cps(0) if RG else kv_cps(0)):
            c.start()

        def zero(i, c):
            for br in range(2):
                acc[br, pl.ds(pl.multiple_of(i * SQ, SQ), SQ)] = jnp.zeros((SQ, D), f32)
            return c
        lax.fori_loop(0, B, zero, 0)

        def w_step(g):
            for c in w_cps(g):
                c.wait()

            @pl.when(g + 1 < NG)
            def _():
                for c in w_cps(g + 1):
                    c.start()

        if RG:
            def pre(r, c):
                for cp in x_cps(r) + rkv_cps(r):
                    cp.start()
                return c
            lax.fori_loop(1, LOOK, pre, 0)

            def ramp_outer(g, carry):
                w_step(g)

                def inner(rr, c):
                    r = g * (NB * RPB) + rr
                    it = r >> LR
                    j = r & (RPB - 1)

                    @pl.when(g == 0)
                    def _():
                        for cp in x_cps(rr):
                            cp.wait()
                    for cp in rkv_cps(r):
                        cp.wait()

                    def mid():
                        nx = r + LOOK

                        @pl.when(nx < NB * RPB)
                        def _():
                            for cp in x_cps(nx):
                                cp.start()

                        @pl.when(nx < NR)
                        def _():
                            for cp in rkv_cps(nx):
                                cp.start()

                        @pl.when(jnp.logical_and(nx >= NR, j == 0))
                        def _():
                            for cp in kv_cps(nx >> LR):
                                cp.start()
                    compute(RB, it & (NS - 1), j * RB, rr * RB, g & 1, rorder, mid, 1, lambda br, j, t: None)
                    return c
                lax.fori_loop(0, NB * RPB, inner, 0)
                return carry
            lax.fori_loop(0, RG, ramp_outer, 0)
        else:
            raise NotImplementedError

        def outer(g, carry):
            w_step(g)

            def inner(bi, c):
                it = g * NB + bi
                for cp in kv_cps(it):
                    cp.wait()

                @pl.when(jnp.logical_and(g == NG - 1, bi > 1))
                def _():
                    for br in range(2):
                        for j in range(osplit):
                            o_cp(bi - 2, br, j).wait()

                def mid():
                    @pl.when(it + NS - 1 < NIT)
                    def _():
                        for cp in kv_cps(it + NS - 1):
                            cp.start()

                def emit(br, j, t):
                    obuf[bi & 1, br, pl.ds(j * OB * SQ, OB * SQ)] = t.astype(bf16)

                    @pl.when(g == NG - 1)
                    def _():
                        o_cp(bi, br, j).start()
                compute(BB, it & (NS - 1), 0, bi * BB, g & 1, order, mid, osplit, emit)
                return c
            lax.fori_loop(0, NB, inner, 0)
            return carry

        lax.fori_loop(RG, NG, outer, 0)
        for bi in (NB - 2, NB - 1):
            for br in range(2):
                for j in range(osplit):
                    o_cp(bi, br, j).wait()

    @jax.jit
    def f(A_x, A_k, A_v, A_wq, A_wo, B_x, B_k, B_v, B_wq, B_wo):
        def t(a):
            return jnp.swapaxes(a, 2, 3).reshape(B, NG_ALL, NP, 2 * DH, SK)
        any_ = pl.BlockSpec(memory_space=pl.ANY)
        per = [pltpu.VMEM((B * SQ, D), bf16), pltpu.VMEM((NS, BB, NP, 2 * DH, SK), bf16),
               pltpu.VMEM((NS, BB, NP, 2 * DH, SK), bf16), pltpu.VMEM((2, D, W), bf16), pltpu.VMEM((2, W, D), bf16)]
        DMA = pltpu.SemaphoreType.DMA
        out = pl.pallas_call(
            kern,
            in_specs=[any_] * 10,
            out_specs=any_,
            out_shape=jax.ShapeDtypeStruct((B * SQ, 2 * D), bf16),
            scratch_shapes=per + per + [
                pltpu.VMEM((2, B * SQ, D), f32), pltpu.VMEM((2, 2, BB * SQ, D), bf16),
                DMA((2, 2, NS)), DMA((2, 2, NS, RPB)), DMA((2, B // RB)), DMA((2, 2, 2)), DMA((2, 2, osplit))],
            compiler_params=pltpu.CompilerParams(vmem_limit_bytes=120 * 2 ** 20, flags=flags),
        )(A_x.reshape(B * SQ, D), t(A_k), t(A_v), A_wq, A_wo.reshape(NG_ALL, W, D),
          B_x.reshape(B * SQ, D), t(B_k), t(B_v), B_wq, B_wo.reshape(NG_ALL, W, D))
        return out.reshape(B, SQ, 2 * D)
    return f


_impl = make(osplit=4)


@jax.jit
def pallas_concat_heads__gqa_block_cached__mha_block_cached__near_ridge_kernel(
    A_x, A_k_cache, A_v_cache, A_wq, A_wo,
    B_x, B_k_cache, B_v_cache, B_wq, B_wo,
):
    return _impl(A_x, A_k_cache, A_v_cache, A_wq, A_wo,
                 B_x, B_k_cache, B_v_cache, B_wq, B_wo)
```

```python
import jax
import jax.numpy as jnp
import numpy as np
from jax import lax
from jax.experimental import pallas as pl
from jax.experimental.pallas import tpu as pltpu

_LANES = 128
_SB = 8
_NT = (((1,), (1,)), ((), ()))
_X, _K, _V, _WQ, _WO = range(5)


def _dot(a, b):
    return jnp.dot(a, b, preferred_element_type=jnp.float32)


def _dot_nt(a, b):
    return lax.dot_general(a, b, _NT, preferred_element_type=jnp.float32)


def _softmax_parts(s):
    e = jnp.exp2(s - jnp.max(s, axis=1, keepdims=True))
    return e.astype(jnp.bfloat16), 1.0 / jnp.sum(e, axis=1, keepdims=True)


@jax.jit
def pallas_concat_heads__gqa_block_cached__mha_block_cached__near_ridge_kernel(
    A_x: jax.Array,
    A_k_cache: jax.Array,
    A_v_cache: jax.Array,
    A_wq: jax.Array,
    A_wo: jax.Array,
    B_x: jax.Array,
    B_k_cache: jax.Array,
    B_v_cache: jax.Array,
    B_wq: jax.Array,
    B_wo: jax.Array,
):
    f32, bf16 = jnp.float32, jnp.bfloat16
    B, SQ, D = A_x.shape
    _, H, SK, DH = A_k_cache.shape
    assert B_x.shape == A_x.shape and B_k_cache.shape == A_k_cache.shape
    assert A_wq.shape == (D, H * DH) and B_wq.shape == (D, H * DH)
    assert 2 * DH == 3 * _LANES and H % 2 == 0 and SQ > _LANES and B == 2 * _SB

    T = _LANES
    W = 2 * DH
    NG = H // 2
    NB = B // _SB
    NIT = NG * NB
    M = _SB * SQ
    HB = _SB // 2
    q_scale = float(DH ** -0.5 * np.log2(np.e))
    whole, halves = ((0, _SB),), ((0, HB), (HB, HB))
    pieces = {(0, _K): whole, (1, _K): whole, (0, _V): whole, (1, _V): halves}

    def kernel(xa, ka, va, wqa, woa, xb, kb, vb, wqb, wob, o_hbm,
               vm, acc, obuf, sems, osems):
        hbm = ((xa, ka, va, wqa, woa), (xb, kb, vb, wqb, wob))

        def x_copy(br, bi):
            return pltpu.make_async_copy(
                hbm[br][_X].at[bi], vm[br][_X].at[bi], sems[br][_X].at[bi])

        def kv_copy(br, kv, it, j):
            first, n = pieces[br, kv][j]
            g, bi, slot = it >> 1, it & 1, it & 1
            return pltpu.make_async_copy(
                hbm[br][kv].at[pl.ds(bi * _SB + first, n), g],
                vm[br][kv].at[slot, pl.ds(first, n)],
                sems[br][kv].at[slot, j])

        def wq_copy(br, g):
            col = g * W if isinstance(g, int) else pl.multiple_of(g * W, W)
            return pltpu.make_async_copy(
                hbm[br][_WQ].at[:, pl.ds(col, W)], vm[br][_WQ].at[g & 1],
                sems[br][_WQ].at[g & 1])

        def wo_copy(br, g):
            return pltpu.make_async_copy(
                hbm[br][_WO].at[g], vm[br][_WO].at[g & 1], sems[br][_WO].at[g & 1])

        def out_copy(br, bi, j):
            rows = pl.ds(j * HB * SQ, HB * SQ)
            return pltpu.make_async_copy(
                obuf.at[br, bi, rows], o_hbm.at[bi, rows, pl.ds(br * D, D)],
                osems[br][j].at[bi])

        first_copies = [wq_copy(0, 0), x_copy(0, 0), wq_copy(1, 0), x_copy(1, 0)]
        first_copies += [kv_copy(br, kv, 0, j) for kv in (_K, _V) for br in range(2)
                         for j in range(len(pieces[br, kv]))]
        first_copies += [wo_copy(0, 0), wo_copy(1, 0)]

        def start_first(i, carry):
            for n, copy in enumerate(first_copies):
                pl.when(i == n)(copy.start)
            return carry

        lax.fori_loop(0, len(first_copies), start_first, 0)

        def zero_acc(i, carry):
            rows = pl.ds(pl.multiple_of(i * SQ, SQ), SQ)
            for br in range(2):
                for bi in range(NB):
                    acc[br, bi, rows] = jnp.zeros((SQ, D), f32)
            return carry

        lax.fori_loop(0, _SB, zero_acc, 0)

        def step(it, carry):
            g, bi, slot = it >> 1, it & 1, it & 1
            wslot = g & 1
            new_pair = bi == 0
            fetch_weights = jnp.logical_and(new_pair, g + 1 < NG)
            lo = lax.broadcasted_iota(jnp.int32, (SQ, T), 1) < T // 2

            def prefetch(br, kv):
                @pl.when(it + 1 < NIT)
                def _():
                    for j in range(len(pieces[br, kv])):
                        kv_copy(br, kv, it + 1, j).start()

            def project_q(br):
                pl.when(new_pair)(lambda: wq_copy(br, g).wait())
                pl.when(g == 0)(lambda: x_copy(br, bi).wait())
                q = _dot(vm[br][_X][bi], vm[br][_WQ][wslot]) * q_scale
                pl.when(it + 1 < NB)(lambda: x_copy(br, it + 1).start())
                pl.when(fetch_weights)(lambda: wq_copy(br, g + 1).start())
                return q

            def probabilities(br, q_all):
                kt = vm[br][_K]
                out = []
                prefetch(br, _K)
                for j, (first, n) in enumerate(pieces[br, _K]):
                    kv_copy(br, _K, it, j).wait()
                    for b in range(first, first + n):
                        q = q_all[b * SQ:(b + 1) * SQ]
                        t0 = q[:, 0:T].astype(bf16)
                        t1 = q[:, T:2 * T]
                        t2 = q[:, 2 * T:W].astype(bf16)
                        t1_h0 = jnp.where(lo, t1, 0.0).astype(bf16)
                        t1_h1 = jnp.where(lo, 0.0, t1).astype(bf16)
                        s0 = _dot(jnp.concatenate([t0, t1_h0], axis=1),
                                  kt[slot, b, 0:2 * T, :])
                        s1 = _dot(jnp.concatenate([t1_h1, t2], axis=1),
                                  kt[slot, b, T:W, :])
                        out.append(_softmax_parts(s0) + _softmax_parts(s1))
                return out

            def attend(br, probs):
                vt = vm[br][_V]
                out = []
                prefetch(br, _V)
                for j, (first, n) in enumerate(pieces[br, _V]):
                    kv_copy(br, _V, it, j).wait()
                    for b in range(first, first + n):
                        p0, r0, p1, r1 = probs[b]
                        left = _dot_nt(p0, vt[slot, b, 0:T, :]) * r0
                        mid0_t = _dot_nt(vt[slot, b, T:DH, :], p0[0:T])
                        right = _dot_nt(p1, vt[slot, b, 2 * T:W, :]) * r1
                        rest = _dot_nt(jnp.concatenate([p0[T:SQ], p1[T:SQ]], axis=0),
                                       vt[slot, b, T:2 * T, :])
                        mid1_t = _dot_nt(vt[slot, b, DH:2 * T, :], p1[0:T])
                        mid_top = jnp.concatenate([mid0_t, mid1_t], axis=0).T
                        mid_bottom = jnp.where(
                            lo[0:SQ - T], rest[0:SQ - T], rest[SQ - T:])
                        mid = (jnp.concatenate([mid_top, mid_bottom], axis=0)
                               * jnp.where(lo, r0, r1))
                        out.append(
                            jnp.concatenate([left, mid, right], axis=1).astype(bf16))
                return out

            def project_out(br, heads):
                pl.when(fetch_weights)(lambda: wo_copy(br, g + 1).start())
                pl.when(new_pair)(lambda: wo_copy(br, g).wait())
                for j in range(2):
                    rows = slice(j * HB * SQ, (j + 1) * HB * SQ)
                    o = jnp.concatenate(heads[j * HB:(j + 1) * HB], axis=0)
                    total = acc[br, bi, rows] + _dot(o, vm[br][_WO][wslot])
                    acc[br, bi, rows] = total
                    obuf[br, bi, rows] = total.astype(bf16)
                    pl.when(g == NG - 1)(out_copy(br, bi, j).start)

            q = [project_q(br) for br in range(2)]
            probs = [probabilities(br, q[br]) for br in range(2)]
            heads = [attend(br, probs[br]) for br in range(2)]
            for br in range(2):
                project_out(br, heads[br])
            return carry

        lax.fori_loop(0, NIT, step, 0)

        for bi in range(NB):
            for br in range(2):
                for j in range(2):
                    out_copy(br, bi, j).wait()

    def pairs(cache):
        return jnp.swapaxes(cache, 2, 3).reshape(B, NG, W, SK)

    dma = pltpu.SemaphoreType.DMA
    in_hbm = pl.BlockSpec(memory_space=pl.ANY)
    buffers = [[
        pltpu.VMEM((NB, M, D), bf16),
        pltpu.VMEM((2, _SB, W, SK), bf16),
        pltpu.VMEM((2, _SB, W, SK), bf16),
        pltpu.VMEM((2, D, W), bf16),
        pltpu.VMEM((2, W, D), bf16),
    ] for br in range(2)]
    sems = [[
        dma((NB,)),
        dma((2, len(pieces[br, _K]))),
        dma((2, len(pieces[br, _V]))),
        dma((2,)),
        dma((2,)),
    ] for br in range(2)]
    out_sems = [[dma((NB,)) for j in range(2)] for br in range(2)]

    out = pl.pallas_call(
        kernel,
        in_specs=[in_hbm] * 10,
        out_specs=in_hbm,
        out_shape=jax.ShapeDtypeStruct((NB, M, 2 * D), bf16),
        scratch_shapes=[
            buffers,
            pltpu.VMEM((2, NB, M, D), f32),
            pltpu.VMEM((2, NB, M, D), bf16),
            sems,
            out_sems,
        ],
        compiler_params=pltpu.CompilerParams(
            vmem_limit_bytes=120 * 2 ** 20,
            flags={"XLA_TPU_RESCHEDULE_DMA_DONES": True},
        ),
    )(
        A_x.reshape(NB, M, D), pairs(A_k_cache), pairs(A_v_cache),
        A_wq, A_wo.reshape(NG, W, D),
        B_x.reshape(NB, M, D), pairs(B_k_cache), pairs(B_v_cache),
        B_wq, B_wo.reshape(NG, W, D),
    )
    return out.reshape(B, SQ, 2 * D)
```
